```python
import os as _os
_os.environ.setdefault("JAX_PLATFORMS", "cpu")
import jax
import jax.numpy as jnp

def _softmax(x, axis=-1):
    return jax.nn.softmax(x, axis=axis)
def _gelu(x):
    return jax.nn.gelu(x, approximate=True)
def _silu(x):
    return jax.nn.silu(x)
def _sigmoid(x):
    return jax.nn.sigmoid(x)
def _layernorm(x, axis=-1, eps=1e-5):
    m = jnp.mean(x, axis=axis, keepdims=True)
    v = jnp.var(x, axis=axis, keepdims=True)
    return (x - m) / jnp.sqrt(v + eps)
def _scatter_add(tgt, idx, src, axis=0):
    return tgt.at[idx].add(src)
def _segment_sum(src, seg, n):
    return jax.ops.segment_sum(src, seg, n)
class _Rng:
    def __init__(self, key):
        self._k = key
    def _next(self):
        self._k, sub = jax.random.split(self._k)
        return sub
    def normal(self, shape):
        return jax.random.normal(self._next(), shape, dtype=jnp.bfloat16)
    def randint(self, lo, hi, shape):
        return jax.random.randint(self._next(), shape, lo, hi, dtype=jnp.int32)
    def uniform(self, shape, lo=0.0, hi=1.0):
        return jax.random.uniform(self._next(), shape, jnp.bfloat16, lo, hi)
    def permutation(self, n):
        return jax.random.permutation(self._next(), n)


kernel_name = 'standalone__mha_softmax__prompt'

def setup_inputs():
    _rng = _Rng(jax.random.key(int.from_bytes(__import__("os").urandom(4), "little")))
    _w = (lambda a: (lambda t: t.astype(jnp.bfloat16) if jnp.issubdtype(t.dtype, jnp.floating) else t)(jnp.asarray(a)))
    B, H, Sq, Sk, D = 1, 32, 2048, 2048, 192
    return {
        "q": _w((lambda *s: _rng.normal(s) * 0.4)(B, H, Sq, D)),
        "k": _w((lambda *s: _rng.normal(s) * 0.4)(B, H, Sk, D)),
        "v": _w((lambda *s: _rng.normal(s) * 0.05)(B, H, Sk, D)),
    }

def reference(q, k, v):
    scale = q.shape[-1] ** -0.5
    scores = jnp.einsum("bhqd,bhkd->bhqk", q, k) * scale
    p = _softmax(scores, axis=-1)
    return jnp.einsum("bhqk,bhkd->bhqd", p, v)
```

```python
import functools
import jax
import jax.numpy as jnp
from jax import lax
import jax.experimental.pallas as pl
import jax.experimental.pallas.tpu as pltpu

LOG2E = 1.4426950408889634
F32 = jnp.float32
BF16 = jnp.bfloat16


def _kernel(qt_ref, kt_ref, vt_ref, ot_ref, ka_ref, kb_ref, kc_ref, vs_ref, s_ref, *, bq, ck, c, lag, da, dl):
    D, Sq = qt_ref.shape
    Sk = kt_ref.shape[1]
    T = D // 3
    nq = Sq // bq
    hb = bq // 2
    nc = Sk // ck
    ns = 3

    ka = kt_ref[0:2 * T, :].T
    kb = jnp.concatenate([kt_ref[2 * T:3 * T, :], kt_ref[0:T, :]], axis=0).T
    lane = lax.broadcasted_iota(jnp.int32, ka.shape, 1)
    ka_ref[...] = ka
    kb_ref[...] = kb
    kc_ref[...] = jnp.where(lane < T, kb, ka)
    vs_ref[...] = vt_ref[...]

    def weights(j):
        qa = qt_ref[:, j * bq:j * bq + hb]
        qb = qt_ref[:, j * bq + hb:(j + 1) * bq]
        qa1, qa2, qa3 = qa[0:T], qa[T:2 * T], qa[2 * T:3 * T]
        qb1, qb2, qb3 = qb[0:T], qb[T:2 * T], qb[2 * T:3 * T]
        d3 = (qa3.astype(F32) - qb3.astype(F32)).astype(BF16)
        d2 = (qb2.astype(F32) - qa2.astype(F32)).astype(BF16)
        w1 = jnp.concatenate([qb3, qa2], axis=0)
        w2 = jnp.concatenate([d3, qa1], axis=0)
        w3 = jnp.concatenate([qb1, d2], axis=0)
        return w1, w2, w3

    def a_chunk(j, ci, w, mrun):
        w1, w2, w3 = w
        rows = slice(ci * ck, (ci + 1) * ck)
        p1 = jnp.dot(kc_ref[rows, :], w1, preferred_element_type=F32)
        p2 = jnp.dot(kb_ref[rows, :], w2, preferred_element_type=F32)
        p3 = jnp.dot(ka_ref[rows, :], w3, preferred_element_type=F32)
        sa = p1 + p2
        sb = p1 + p3
        s_ref[j % ns, rows, 0:hb] = sa
        s_ref[j % ns, rows, hb:bq] = sb
        ma = jnp.max(sa.reshape(ck // 8, 8, hb), axis=0)
        mb = jnp.max(sb.reshape(ck // 8, 8, hb), axis=0)
        mm = jnp.concatenate([ma, mb], axis=1)
        return mm if mrun is None else jnp.maximum(mrun, mm)

    def b_chunk(j, ci, m8, lrun, acc):
        rows = slice(ci * ck, (ci + 1) * ck)
        s = s_ref[j % ns, rows, :].reshape(ck // 8, 8, bq)
        p = jnp.exp2((s - m8[None]) * c)
        ls = jnp.sum(p, axis=0)
        o = jnp.dot(vs_ref[:, rows], p.reshape(ck, bq).astype(BF16), preferred_element_type=F32)
        return (ls if lrun is None else lrun + ls), (o if acc is None else acc + o)

    def tie(m8, x):
        return jnp.maximum(m8, jnp.minimum(x, m8))

    total = nq * nc
    ms = {}
    mhist = {}
    lhist = {}
    mrun = None
    lrun = acc = None
    w = None
    for g in range(total + lag):
        if g < total:
            j, ci = divmod(g, nc)
            if ci == 0:
                w = weights(j)
                mrun = None
            mrun = a_chunk(j, ci, w, mrun)
            mhist[g] = mrun
            if ci == nc - 1:
                ms[j] = jnp.broadcast_to(jnp.max(mrun, axis=0, keepdims=True), (8, bq))
        gb = g - lag
        if gb >= 0:
            j, ci = divmod(gb, nc)
            if ci == 0:
                lrun = acc = None
            m8 = ms[j]
            if da is not None and (g - da) in mhist:
                m8 = tie(m8, mhist[g - da])
            if dl is not None and (gb - dl) in lhist:
                m8 = tie(m8, lhist[gb - dl])
            lrun, acc = b_chunk(j, ci, m8, lrun, acc)
            lhist[gb] = lrun
            if ci == nc - 1:
                l = jnp.sum(lrun, axis=0, keepdims=True)
                ot_ref[:, j * bq:(j + 1) * bq] = (acc * (1.0 / l)).astype(ot_ref.dtype)


@functools.partial(jax.jit, static_argnames=('bq', 'ck', 'lag', 'da', 'dl'))
def pallas_standalone__mha_softmax__prompt_kernel(q, k, v, bq=256, ck=128, lag=18, da=2, dl=2):
    B, H, Sq, D = q.shape
    Sk = k.shape[2]
    qt = jnp.swapaxes(q, 2, 3).reshape(B * H, D, Sq)
    kt = jnp.swapaxes(k, 2, 3).reshape(B * H, D, Sk)
    vt = jnp.swapaxes(v, 2, 3).reshape(B * H, D, Sk)
    c = (D ** -0.5) * LOG2E
    ot = pl.pallas_call(
        functools.partial(_kernel, bq=bq, ck=ck, c=c, lag=lag, da=da, dl=dl),
        grid=(B * H,),
        in_specs=[
            pl.BlockSpec((None, D, Sq), lambda h: (h, 0, 0)),
            pl.BlockSpec((None, D, Sk), lambda h: (h, 0, 0)),
            pl.BlockSpec((None, D, Sk), lambda h: (h, 0, 0)),
        ],
        out_specs=pl.BlockSpec((None, D, Sq), lambda h: (h, 0, 0)),
        out_shape=jax.ShapeDtypeStruct((B * H, D, Sq), q.dtype),
        scratch_shapes=[
            pltpu.VMEM((Sk, 128), BF16),
            pltpu.VMEM((Sk, 128), BF16),
            pltpu.VMEM((Sk, 128), BF16),
            pltpu.VMEM((D, Sk), BF16),
            pltpu.VMEM((3, Sk, bq), F32),
        ],
        compiler_params=pltpu.CompilerParams(
            dimension_semantics=("arbitrary",),
            vmem_limit_bytes=100 * 1024 * 1024),
    )(qt, kt, vt)
    return jnp.swapaxes(ot.reshape(B, H, D, Sq), 2, 3)
```

```python
import functools
import jax
import jax.numpy as jnp
from jax import lax
import jax.experimental.pallas as pl
import jax.experimental.pallas.tpu as pltpu

LOG2E = 1.4426950408889634
F32 = jnp.float32
BF16 = jnp.bfloat16
U32 = jnp.uint32


def _kernel(q_hbm, k_hbm, v_hbm, o_hbm,
            qk_buf, vbuf, obuf, o0buf, ka_ref, kb_ref, kc_ref, sx_ref, mx_ref, wx_ref,
            sem_qk, sem_v, sem_o, sem_p, *, bq, ck, c, lag, da, dl, dacc, start_at, sb, edacc, ksplit, kearly, vearly):
    BH, D, Sq = q_hbm.shape
    Sk = k_hbm.shape[2]
    T = D // 3
    nq = Sq // bq
    hb = bq // 2
    nc = Sk // ck
    total = nq * nc
    s0 = sb * nc
    nh = -(-(s0 + lag) // nc)
    qh = nh * bq
    nsteps = BH - 1

    def start_set(head, head_next, slot, vslot):
        pltpu.make_async_copy(q_hbm.at[head, :, pl.ds(qh, Sq - qh)],
                              qk_buf.at[slot, :, pl.ds(qh, Sq - qh)], sem_qk.at[slot]).start()
        pltpu.make_async_copy(k_hbm.at[head_next],
                              qk_buf.at[slot, :, pl.ds(Sq, Sk)], sem_qk.at[slot]).start()
        pltpu.make_async_copy(q_hbm.at[head_next, :, pl.ds(0, qh)],
                              qk_buf.at[slot, :, pl.ds(0, qh)], sem_qk.at[slot]).start()
        pltpu.make_async_copy(v_hbm.at[head_next], vbuf.at[vslot], sem_v.at[vslot]).start()

    def wait_set(slot, vslot):
        pltpu.make_async_copy(qk_buf.at[slot], qk_buf.at[slot], sem_qk.at[slot]).wait()
        pltpu.make_async_copy(vbuf.at[vslot], vbuf.at[vslot], sem_v.at[vslot]).wait()

    def o_start(src, head, j, sem):
        pltpu.make_async_copy(src, o_hbm.at[head, :, pl.ds(j * bq, bq)], sem).start()

    def o_wait(slot, nblk):
        part = obuf.at[slot, :, pl.ds(0, nblk * bq)]
        pltpu.make_async_copy(part, part, sem_o.at[slot]).wait()

    def k_prep(src_ref, ci):
        cols = slice(Sq + ci * ck, Sq + (ci + 1) * ck)
        ka = src_ref[0:2 * T, cols].T
        kb = jnp.concatenate([src_ref[2 * T:3 * T, cols], src_ref[0:T, cols]], axis=0).T
        prow = slice(ci * ck // 2, (ci + 1) * ck // 2)
        ka = pltpu.bitcast(ka, U32)
        kb = pltpu.bitcast(kb, U32)
        lane = lax.broadcasted_iota(jnp.int32, ka.shape, 1)
        ka_ref[prow, :] = ka
        kb_ref[prow, :] = kb
        kc_ref[prow, :] = jnp.where(lane < T, kb, ka)

    def weights(src_ref, j):
        qa = src_ref[:, j * bq:j * bq + hb]
        qb = src_ref[:, j * bq + hb:(j + 1) * bq]
        qa1, qa2, qa3 = qa[0:T], qa[T:2 * T], qa[2 * T:3 * T]
        qb1, qb2, qb3 = qb[0:T], qb[T:2 * T], qb[2 * T:3 * T]
        d3 = (qa3.astype(F32) - qb3.astype(F32)).astype(BF16)
        d2 = (qb2.astype(F32) - qa2.astype(F32)).astype(BF16)
        w1 = jnp.concatenate([qb3, qa2], axis=0)
        w2 = jnp.concatenate([d3, qa1], axis=0)
        w3 = jnp.concatenate([qb1, d2], axis=0)
        return w1, w2, w3

    def a_chunk(ci, w, mrun):
        w1, w2, w3 = w
        rows = slice(ci * ck // 2, (ci + 1) * ck // 2)
        p1 = jnp.dot(pltpu.bitcast(kc_ref[rows, :], BF16), w1, preferred_element_type=F32)
        p2 = jnp.dot(pltpu.bitcast(kb_ref[rows, :], BF16), w2, preferred_element_type=F32)
        p3 = jnp.dot(pltpu.bitcast(ka_ref[rows, :], BF16), w3, preferred_element_type=F32)
        s = jnp.concatenate([p1 + p2, p1 + p3], axis=1)
        mm = jnp.max(s.reshape(ck // 8, 8, bq), axis=0)
        return s, (mm if mrun is None else jnp.maximum(mrun, mm))

    def b_chunk(v_ref, ci, s, m8, lrun, acc):
        rows = slice(ci * ck, (ci + 1) * ck)
        p = jnp.exp2((s.reshape(ck // 8, 8, bq) - m8[None]) * c)
        ls = jnp.sum(p, axis=0)
        o = jnp.dot(v_ref[:, rows], p.reshape(ck, bq).astype(BF16), preferred_element_type=F32)
        return (ls if lrun is None else lrun + ls), (o if acc is None else acc + o)

    def tie(m8, x):
        return jnp.maximum(m8, jnp.minimum(x, m8))

    def finish_m(mrun):
        return jnp.broadcast_to(jnp.max(mrun, axis=0, keepdims=True), (8, bq))

    def segment(g0, g1, a_end, q_ref, prep_next, v_of, out, hooks, load_state):
        ms, ss, mhist, lhist, ahist = {}, {}, {}, {}, {}
        mrun = w = None
        if load_state:
            b0 = g0 // nc
            for i in range(lag // nc):
                ms[b0 + i] = mx_ref[i]
            if lag % nc:
                mrun = mx_ref[lag // nc]
                w = tuple(pltpu.bitcast(wx_ref[i], BF16) for i in range(3))
        lrun = acc = None
        for g in range(g0, g1):
            if g in hooks:
                hooks[g]()
            ga = g + lag
            if ga < a_end:
                blk, ci = divmod(ga, nc)
                if ci == 0:
                    w = weights(q_ref, blk % nq)
                    mrun = None
                s, mrun = a_chunk(ci, w, mrun)
                mhist[g] = mrun
                if ga < g1:
                    ss[ga] = s
                else:
                    sx_ref[ga - g1] = s
                if ci == nc - 1:
                    if ga < g1:
                        ms[blk] = finish_m(mrun)
                    else:
                        mx_ref[blk - g1 // nc] = finish_m(mrun)
                elif g == g1 - 1:
                    mx_ref[blk - g1 // nc] = mrun
                    for i in range(3):
                        wx_ref[i] = pltpu.bitcast(w[i], U32)
                if blk == nq - 1 and prep_next:
                    k_prep(q_ref, ci)
            if g >= 0:
                blk, ci = divmod(g, nc)
                if ci == 0:
                    lrun = acc = None
                m8 = ms[blk]
                if (g - da) in mhist:
                    m8 = tie(m8, mhist[g - da])
                if (g - dl) in lhist:
                    m8 = tie(m8, lhist[g - dl])
                dd = dacc if ga < a_end else edacc
                if dd and (g - dd) in ahist:
                    m8 = tie(m8, ahist[g - dd])
                s = ss.pop(g) if g in ss else sx_ref[g - g0]
                lrun, acc = b_chunk(v_of(blk), ci, s, m8, lrun, acc)
                lhist[g] = lrun
                ahist[g] = acc[D - 8:D]
                if ci == nc - 1:
                    l = jnp.sum(lrun, axis=0, keepdims=True)
                    out(blk, (acc * (1.0 / l)).astype(BF16))

    q0 = 2 * bq
    kp = Sk // ksplit
    cp_q0 = pltpu.make_async_copy(q_hbm.at[0, :, pl.ds(0, q0)], qk_buf.at[1, :, pl.ds(0, q0)], sem_p.at[0])
    cp_q1 = pltpu.make_async_copy(q_hbm.at[0, :, pl.ds(q0, qh - q0)], qk_buf.at[1, :, pl.ds(q0, qh - q0)], sem_p.at[1])
    cp_k = [pltpu.make_async_copy(k_hbm.at[0, :, pl.ds(i * kp, kp)], qk_buf.at[1, :, pl.ds(Sq + i * kp, kp)], sem_p.at[3 + i])
            for i in range(ksplit)]
    cp_v = pltpu.make_async_copy(v_hbm.at[0], vbuf.at[0], sem_v.at[0])
    cp_q0.start()
    cp_k[0].start()
    for i in range(1, ksplit):
        cp_k[i].start()
    cp_q0.wait()
    cp_v.start()
    cp_q1.start()

    def pro_prep(i):
        def f():
            cp_k[i].wait()
            for ci in range(i * nc // ksplit, (i + 1) * nc // ksplit):
                k_prep(qk_buf.at[1], ci)
        return f

    def pro_v():
        cp_q1.wait()
        start_set(0, 1, 0, 1)
        cp_v.wait()

    def pro_out(blk, val):
        o0buf[:, blk * bq:(blk + 1) * bq] = val
        o_start(o0buf.at[:, pl.ds(blk * bq, bq)], 0, blk, sem_p.at[2])

    hooks = {-lag + max(0, i * nc // ksplit - kearly): pro_prep(i) for i in range(ksplit)}
    hooks[-vearly] = pro_v
    segment(-lag, s0, total, qk_buf.at[1], False, lambda blk: vbuf.at[0], pro_out, hooks, False)

    def step(h, carry):
        cur = h & 1
        oth = 1 - cur
        h1 = h + 1
        h2 = jnp.minimum(h + 2, BH - 1)
        v0 = h & 3
        v1 = (h + 1) & 3
        v2 = (h + 2) & 3

        @pl.when(h >= 2)
        def _():
            o_wait(cur, nq)

        wait_set(cur, v1)

        def out_main(blk, val):
            pos = blk - sb
            obuf[cur, :, pos * bq:(pos + 1) * bq] = val
            o_start(obuf.at[cur, :, pl.ds(pos * bq, bq)], h1 if blk >= nq else h, blk % nq, sem_o.at[cur])

        segment(s0, total + s0, 2 * total, qk_buf.at[cur], True,
                lambda blk: vbuf.at[v1] if blk >= nq else vbuf.at[v0], out_main,
                {s0 + start_at: lambda: start_set(h1, h2, oth, v2)}, True)
        return carry

    lax.fori_loop(0, nsteps, step, 0)

    cur = nsteps & 1
    o_wait(cur, nq)
    wait_set(cur, (nsteps + 1) & 3)

    def epi_out(blk, val):
        pos = blk - sb
        obuf[cur, :, pos * bq:(pos + 1) * bq] = val
        o_start(obuf.at[cur, :, pl.ds(pos * bq, bq)], BH - 1, blk, sem_o.at[cur])

    segment(s0, total, total, qk_buf.at[cur], False, lambda blk: vbuf.at[nsteps & 3], epi_out, {}, True)
    pltpu.make_async_copy(o0buf, o0buf, sem_p.at[2]).wait()
    o_wait(1 - cur, nq)
    o_wait(cur, nq - sb)


@functools.partial(jax.jit, static_argnames=('bq', 'ck', 'lag', 'da', 'dl', 'dacc', 'start_at', 'sb', 'nobc', 'edacc', 'ksplit', 'kearly', 'vearly'))
def pallas_standalone__mha_softmax__prompt_kernel(q, k, v, bq=256, ck=128, lag=18, da=3, dl=2, dacc=3, start_at=4, sb=2, nobc=True, edacc=6, ksplit=2, kearly=3, vearly=0):
    B, H, Sq, D = q.shape
    Sk = k.shape[2]
    BH = B * H
    assert BH >= 3
    qt = jnp.swapaxes(q, 2, 3).reshape(BH, D, Sq)
    kt = jnp.swapaxes(k, 2, 3).reshape(BH, D, Sk)
    vt = jnp.swapaxes(v, 2, 3).reshape(BH, D, Sk)
    c = (D ** -0.5) * LOG2E
    nc = Sk // ck
    ot = pl.pallas_call(
        functools.partial(_kernel, bq=bq, ck=ck, c=c, lag=lag, da=da, dl=dl, dacc=dacc, start_at=start_at, sb=sb,
                          edacc=edacc, ksplit=ksplit, kearly=kearly, vearly=vearly),
        in_specs=[pl.BlockSpec(memory_space=pl.ANY)] * 3,
        out_specs=pl.BlockSpec(memory_space=pl.ANY),
        out_shape=jax.ShapeDtypeStruct((BH, D, Sq), q.dtype),
        scratch_shapes=[
            pltpu.VMEM((2, D, Sq + Sk), BF16),
            pltpu.VMEM((4, D, Sk), BF16),
            pltpu.VMEM((2, D, Sq), BF16),
            pltpu.VMEM((D, sb * bq), BF16),
            pltpu.VMEM((Sk // 2, 128), U32),
            pltpu.VMEM((Sk // 2, 128), U32),
            pltpu.VMEM((Sk // 2, 128), U32),
            pltpu.VMEM((lag, ck, bq), F32),
            pltpu.VMEM((-(-lag // nc), 8, bq), F32),
            pltpu.VMEM((3, 64, bq // 2), U32),
            pltpu.SemaphoreType.DMA((2,)),
            pltpu.SemaphoreType.DMA((4,)),
            pltpu.SemaphoreType.DMA((2,)),
            pltpu.SemaphoreType.DMA((3 + ksplit,)),
        ],
        compiler_params=pltpu.CompilerParams(
            disable_bounds_checks=nobc,
            vmem_limit_bytes=100 * 1024 * 1024),
    )(qt, kt, vt)
    return jnp.swapaxes(ot.reshape(B, H, D, Sq), 2, 3)
```

```python
import functools

import jax
import jax.numpy as jnp
from jax import lax
import jax.experimental.pallas as pl
import jax.experimental.pallas.tpu as pltpu

LOG2E = 1.4426950408889634
F32 = jnp.float32
BF16 = jnp.bfloat16
U32 = jnp.uint32
I32 = jnp.int32

BQ = 256
CK = 128
LAG = 18
SHIFT = 2
LEAD = 8
DA, DL, DACC, DACC_TAIL = 3, 2, 3, 6
PREP_AT, PREP_GAP = 9, 2
FETCH_AT = 40


def _kernel(q_hbm, k_hbm, v_hbm, o_hbm,
            qk_buf, v_buf, o_buf, o0_buf, ka_ref, kb_ref, kc_ref,
            sx_ref, mx_ref, cx_ref, wx_ref,
            sem_qk, sem_v, sem_o, sem_p, *, c):
    BH, D, Sq = q_hbm.shape
    Sk = k_hbm.shape[2]
    T = D // 3
    hb = BQ // 2
    nq = Sq // BQ
    nc = Sk // CK
    total = nq * nc
    s0 = SHIFT * nc
    nh = -(-(s0 + LAG) // nc)
    qh = nh * BQ
    nsteps = BH - 1

    def start_set(head, head_next, slot, vslot):
        pltpu.make_async_copy(q_hbm.at[head, :, pl.ds(qh, Sq - qh)],
                              qk_buf.at[slot, :, pl.ds(qh, Sq - qh)], sem_qk.at[slot]).start()
        pltpu.make_async_copy(k_hbm.at[head_next],
                              qk_buf.at[slot, :, pl.ds(Sq, Sk)], sem_qk.at[slot]).start()
        pltpu.make_async_copy(q_hbm.at[head_next, :, pl.ds(0, qh)],
                              qk_buf.at[slot, :, pl.ds(0, qh)], sem_qk.at[slot]).start()
        pltpu.make_async_copy(v_hbm.at[head_next], v_buf.at[vslot], sem_v.at[vslot]).start()

    def wait_set(slot, vslot):
        pltpu.make_async_copy(qk_buf.at[slot], qk_buf.at[slot], sem_qk.at[slot]).wait()
        pltpu.make_async_copy(v_buf.at[vslot], v_buf.at[vslot], sem_v.at[vslot]).wait()

    def o_start(src, head, j, sem):
        pltpu.make_async_copy(src, o_hbm.at[head, :, pl.ds(j * BQ, BQ)], sem).start()

    def o_wait(slot, nblk):
        part = o_buf.at[slot, :, pl.ds(0, nblk * BQ)]
        pltpu.make_async_copy(part, part, sem_o.at[slot]).wait()

    def k_prep(src_ref, ci):
        cols = slice(Sq + ci * CK, Sq + (ci + 1) * CK)
        ka = src_ref[0:2 * T, cols].T
        kb = jnp.concatenate([src_ref[2 * T:3 * T, cols], src_ref[0:T, cols]], axis=0).T
        ka = pltpu.bitcast(ka, U32)
        kb = pltpu.bitcast(kb, U32)
        lane = lax.broadcasted_iota(I32, ka.shape, 1)
        rows = slice(ci * CK // 2, (ci + 1) * CK // 2)
        ka_ref[rows, :] = ka
        kb_ref[rows, :] = kb
        kc_ref[rows, :] = jnp.where(lane < T, kb, ka)

    def col_scales(src_ref, j):
        u = pltpu.bitcast(src_ref[:, j * BQ:(j + 1) * BQ], U32)
        hi = pltpu.bitcast(u & jnp.uint32(0xFFFF0000), F32)
        lo = pltpu.bitcast(lax.shift_left(u, jnp.uint32(16)), F32)
        ss = jnp.sum(hi * hi + lo * lo, axis=0, keepdims=True)
        ss = jnp.broadcast_to(ss, (8, BQ))
        e = lax.shift_right_logical(pltpu.bitcast(ss, I32), 24)
        up = pltpu.bitcast(lax.shift_left(190 - e, 23), F32)
        down = pltpu.bitcast(lax.shift_left(64 + e, 23), F32)
        return up, down * c

    def weight(src_ref, j, up, i):
        def part(half, t):
            cols = slice(j * BQ + half * hb, j * BQ + (half + 1) * hb)
            x = src_ref[t * T:(t + 1) * T, cols].astype(F32)
            u = up[:, half * hb:(half + 1) * hb]
            return (x.reshape(T // 8, 8, hb) * u[None]).reshape(T, hb)
        if i == 0:
            w = jnp.concatenate([part(1, 2), part(0, 1)], axis=0)
        elif i == 1:
            w = jnp.concatenate([part(0, 2) - part(1, 2), part(0, 0)], axis=0)
        else:
            w = jnp.concatenate([part(1, 0), part(1, 1) - part(0, 1)], axis=0)
        return w.astype(BF16)

    def a_chunk(ci, w, mrun):
        rows = slice(ci * CK // 2, (ci + 1) * CK // 2)
        p2 = jnp.dot(pltpu.bitcast(kb_ref[rows, :], BF16), w[1], preferred_element_type=F32)
        p1 = jnp.dot(pltpu.bitcast(kc_ref[rows, :], BF16), w[0], preferred_element_type=F32)
        p3 = jnp.dot(pltpu.bitcast(ka_ref[rows, :], BF16), w[2], preferred_element_type=F32)
        s = jnp.concatenate([p1 + p2, p1 + p3], axis=1)
        mm = jnp.max(s.reshape(CK // 8, 8, BQ), axis=0)
        return s, (mm if mrun is None else jnp.maximum(mrun, mm))

    def b_chunk(v_ref, ci, s, m8, c8, lrun, acc):
        p = jnp.exp2((s.reshape(CK // 8, 8, BQ) - m8[None]) * c8[None])
        ls = jnp.sum(p, axis=0)
        o = jnp.dot(v_ref[:, ci * CK:(ci + 1) * CK], p.reshape(CK, BQ).astype(BF16),
                    preferred_element_type=F32)
        return (ls if lrun is None else lrun + ls), (o if acc is None else acc + o)

    def col_max(mrun):
        return jnp.broadcast_to(jnp.max(mrun, axis=0, keepdims=True), (8, BQ))

    def order_after(m8, x):
        if x.dtype == I32:
            mi = pltpu.bitcast(m8, I32)
            return pltpu.bitcast(jnp.maximum(mi, jnp.minimum(x, mi)), F32)
        return jnp.maximum(m8, jnp.minimum(x, m8))

    def fold(w):
        u = jnp.max(pltpu.bitcast(w, I32).reshape(4, 16, hb), axis=0)
        return jnp.concatenate([u[:8], u[8:]], axis=1)

    def segment(ops, g0, g1, q_ref, prep_next, v_of, out, resume):
        ms, ss, cs, scales, wnext = {}, {}, {}, {}, {}
        mhist, lhist, ahist, pend = [], [], [], []
        mrun = w = lrun = acc = None
        if resume:
            for i in range(LAG // nc):
                ms[g0 // nc + i] = mx_ref[i]
            for i in range(-(-LAG // nc)):
                cs[g0 // nc + i] = cx_ref[i]
            mrun = mx_ref[LAG // nc]
            w = tuple(pltpu.bitcast(wx_ref[i], BF16) for i in range(3))
        for op in ops:
            if op[0] == 'H':
                op[1]()
            elif op[0] == 'A':
                ga = op[1]
                blk, ci = divmod(ga, nc)
                if ci == 0:
                    if blk not in scales:
                        scales[blk] = col_scales(q_ref, blk % nq)
                    up, c8 = scales[blk]
                    w = tuple(wnext[i] if i in wnext else weight(q_ref, blk % nq, up, i)
                              for i in range(3))
                    wnext.clear()
                    if ga < g1:
                        cs[blk] = c8
                    else:
                        cx_ref[blk - g1 // nc] = c8
                    mrun = None
                if ci == PREP_AT and ('A', (blk + 1) * nc) in ops:
                    scales[blk + 1] = col_scales(q_ref, (blk + 1) % nq)
                    pend.append(scales[blk + 1][1])
                i, r = divmod(ci - PREP_AT - PREP_GAP, PREP_GAP)
                if r == 0 and 0 <= i < 3 and (blk + 1) in scales:
                    wnext[i] = weight(q_ref, (blk + 1) % nq, scales[blk + 1][0], i)
                    pend.append(fold(wnext[i]))
                s, mrun = a_chunk(ci, w, mrun)
                mhist.append(mrun)
                if ga < g1:
                    ss[ga] = s
                else:
                    sx_ref[ga - g1] = s
                if ci == nc - 1:
                    if ga < g1:
                        ms[blk] = col_max(mrun)
                    else:
                        mx_ref[blk - g1 // nc] = col_max(mrun)
                elif ga == g1 + LAG - 1:
                    mx_ref[blk - g1 // nc] = mrun
                    for i in range(3):
                        wx_ref[i] = pltpu.bitcast(w[i], U32)
                if blk == nq - 1 and prep_next:
                    k_prep(q_ref, ci)
            else:
                g, dacc, da = op[1:]
                blk, ci = divmod(g, nc)
                if ci == 0:
                    lrun = acc = None
                m8 = ms[blk]
                if da is not None and len(mhist) > da:
                    m8 = order_after(m8, mhist[-1 - da])
                if len(lhist) >= DL:
                    m8 = order_after(m8, lhist[-DL])
                while pend:
                    m8 = order_after(m8, pend.pop())
                if len(ahist) >= dacc:
                    m8 = order_after(m8, ahist[-dacc])
                s = ss.pop(g) if g in ss else sx_ref[g - g0]
                lrun, acc = b_chunk(v_of(blk), ci, s, m8, cs[blk], lrun, acc)
                lhist.append(lrun)
                ahist.append(acc[D - 8:D])
                if ci == nc - 1:
                    l = jnp.sum(lrun, axis=0, keepdims=True)
                    out(blk, (acc * (1.0 / l)).astype(BF16))

    q0 = ((LAG + LEAD - 1 - PREP_AT) // nc + 2) * BQ
    kp = Sk // 2
    cp_q0 = pltpu.make_async_copy(q_hbm.at[0, :, pl.ds(0, q0)],
                                  qk_buf.at[1, :, pl.ds(0, q0)], sem_p.at[0])
    cp_q1 = pltpu.make_async_copy(q_hbm.at[0, :, pl.ds(q0, qh - q0)],
                                  qk_buf.at[1, :, pl.ds(q0, qh - q0)], sem_p.at[1])
    cp_k = [pltpu.make_async_copy(k_hbm.at[0, :, pl.ds(i * kp, kp)],
                                  qk_buf.at[1, :, pl.ds(Sq + i * kp, kp)], sem_p.at[3 + i])
            for i in range(2)]
    cp_v = pltpu.make_async_copy(v_hbm.at[0], v_buf.at[0], sem_v.at[0])
    cp_q0.start()
    cp_k[0].start()
    cp_k[1].start()
    cp_q0.wait()
    cp_v.start()
    cp_q1.start()

    def first_k(i):
        def f():
            cp_k[i].wait()
            for ci in range(i * nc // 2, (i + 1) * nc // 2):
                k_prep(qk_buf.at[1], ci)
        return f

    def first_b():
        cp_q1.wait()
        start_set(0, 1, 0, 1)
        cp_v.wait()

    def first_out(blk, val):
        o0_buf[:, blk * BQ:(blk + 1) * BQ] = val
        o_start(o0_buf.at[:, pl.ds(blk * BQ, BQ)], 0, blk, sem_p.at[2])

    ops = [('H', first_k(0))]
    for ga in range(LAG + LEAD):
        if ga == nc // 2 - 3:
            ops.append(('H', first_k(1)))
        ops.append(('A', ga))
    ops.append(('H', first_b))
    ga, g = LAG + LEAD, 0
    while g < s0:
        catch_up = ga - g > LAG
        ops.append(('A', ga))
        ops.append(('B', g, DACC_TAIL if catch_up else DACC, DA))
        ga, g = ga + 1, g + 1
        if catch_up:
            ops.append(('B', g, DACC_TAIL, DA))
            g += 1
    assert ga == s0 + LAG and g == s0
    segment(ops, 0, s0, qk_buf.at[1], False, lambda blk: v_buf.at[0], first_out, False)
    wait_set(0, 1)

    def step(h, carry):
        cur = h & 1
        oth = 1 - cur
        h1 = h + 1
        h2 = jnp.minimum(h + 2, BH - 1)
        v0, v1, v2 = h & 3, (h + 1) & 3, (h + 2) & 3

        def out(blk, val):
            pos = blk - SHIFT
            o_buf[cur, :, pos * BQ:(pos + 1) * BQ] = val
            o_start(o_buf.at[cur, :, pl.ds(pos * BQ, BQ)], h1 if blk >= nq else h, blk % nq,
                    sem_o.at[cur])

        ops = []
        for g in range(s0, total + s0):
            if g == s0 + FETCH_AT:
                ops.append(('H', lambda: start_set(h1, h2, oth, v2)))
            ops.append(('A', g + LAG))
            ops.append(('B', g, DACC, DA))
        segment(ops, s0, total + s0, qk_buf.at[cur], True,
                lambda blk: v_buf.at[v1] if blk >= nq else v_buf.at[v0], out, True)

        @pl.when(h >= 1)
        def _():
            o_wait(oth, nq)

        wait_set(oth, v2)
        return carry

    lax.fori_loop(0, nsteps, step, 0)

    cur = nsteps & 1

    def last_out(blk, val):
        pos = blk - SHIFT
        o_buf[cur, :, pos * BQ:(pos + 1) * BQ] = val
        o_start(o_buf.at[cur, :, pl.ds(pos * BQ, BQ)], BH - 1, blk, sem_o.at[cur])

    ops = []
    for g in range(s0, total):
        if g + LAG < total:
            ops.append(('A', g + LAG))
            ops.append(('B', g, DACC, DA))
        else:
            da = DA - (g + LAG - total + 1)
            ops.append(('B', g, DACC_TAIL, da if da >= 0 else None))
    segment(ops, s0, total, qk_buf.at[cur], False, lambda blk: v_buf.at[nsteps & 3],
            last_out, True)
    pltpu.make_async_copy(o0_buf, o0_buf, sem_p.at[2]).wait()
    o_wait(1 - cur, nq)
    o_wait(cur, nq - SHIFT)


@jax.jit
def pallas_standalone__mha_softmax__prompt_kernel(
    q: jax.Array,
    k: jax.Array,
    v: jax.Array,
):
    B, H, Sq, D = q.shape
    Sk = k.shape[2]
    BH = B * H
    nc = Sk // CK
    nx = -(-LAG // nc)
    assert D == 192 and BH >= 3 and Sq % BQ == 0 and Sk % (2 * CK) == 0
    assert LAG % nc and nc > PREP_AT + 3 * PREP_GAP - 1 and SHIFT + nx < Sq // BQ
    qt = jnp.swapaxes(q, 2, 3).reshape(BH, D, Sq)
    kt = jnp.swapaxes(k, 2, 3).reshape(BH, D, Sk)
    vt = jnp.swapaxes(v, 2, 3).reshape(BH, D, Sk)
    ot = pl.pallas_call(
        functools.partial(_kernel, c=(D ** -0.5) * LOG2E),
        in_specs=[pl.BlockSpec(memory_space=pl.ANY)] * 3,
        out_specs=pl.BlockSpec(memory_space=pl.ANY),
        out_shape=jax.ShapeDtypeStruct((BH, D, Sq), q.dtype),
        scratch_shapes=[
            pltpu.VMEM((2, D, Sq + Sk), BF16),
            pltpu.VMEM((4, D, Sk), BF16),
            pltpu.VMEM((2, D, Sq), BF16),
            pltpu.VMEM((D, SHIFT * BQ), BF16),
            pltpu.VMEM((Sk // 2, 128), U32),
            pltpu.VMEM((Sk // 2, 128), U32),
            pltpu.VMEM((Sk // 2, 128), U32),
            pltpu.VMEM((LAG, CK, BQ), F32),
            pltpu.VMEM((nx, 8, BQ), F32),
            pltpu.VMEM((nx, 8, BQ), F32),
            pltpu.VMEM((3, 64, BQ // 2), U32),
            pltpu.SemaphoreType.DMA((2,)),
            pltpu.SemaphoreType.DMA((4,)),
            pltpu.SemaphoreType.DMA((2,)),
            pltpu.SemaphoreType.DMA((5,)),
        ],
        compiler_params=pltpu.CompilerParams(vmem_limit_bytes=64 * 1024 * 1024),
    )(qt, kt, vt)
    return jnp.swapaxes(ot.reshape(B, H, D, Sq), 2, 3)
```

```python
import functools

import jax
import jax.numpy as jnp
from jax import lax
import jax.experimental.pallas as pl
import jax.experimental.pallas.tpu as pltpu

LOG2E = 1.4426950408889634
F32 = jnp.float32
BF16 = jnp.bfloat16
U32 = jnp.uint32
I32 = jnp.int32

BQ = 256
CK = 128
LAG = 18
SHIFT = 2
LEAD = 6
DA, DL, DACC, DACC_TAIL = 3, 2, 3, 5
PREP_AT, PREP_GAP = 9, 2
FETCH_AT = (2, 3, 4)


def _kernel(q_hbm, k_hbm, v_hbm, o_hbm,
            in_buf, o_buf, o0_buf, ka_ref, kb_ref, kc_ref,
            sx_ref, mx_ref, cx_ref, wx_ref,
            sem_in, sem_o, sem_p, *, c):
    BH, D, Sq = q_hbm.shape
    Sk = k_hbm.shape[2]
    T = D // 3
    hb = BQ // 2
    nq = Sq // BQ
    nc = Sk // CK
    total = nq * nc
    s0 = SHIFT * nc
    nsteps = BH - 1
    ko, vo = Sq, Sq + Sk

    def head_copies(head, slot):
        return [pltpu.make_async_copy(src.at[head], in_buf.at[slot, :, pl.ds(off, n)],
                                      sem_in.at[slot])
                for src, off, n in ((q_hbm, 0, Sq), (k_hbm, ko, Sk), (v_hbm, vo, Sk))]

    def wait_head(slot):
        pltpu.make_async_copy(in_buf.at[slot], in_buf.at[slot], sem_in.at[slot]).wait()

    def o_start(src, head, j, sem):
        pltpu.make_async_copy(src, o_hbm.at[head, :, pl.ds(j * BQ, BQ)], sem).start()

    def o_wait(slot, nblk):
        part = o_buf.at[slot, :, pl.ds(0, nblk * BQ)]
        pltpu.make_async_copy(part, part, sem_o.at[slot]).wait()

    def k_prep(src_ref, ci):
        cols = slice(ko + ci * CK, ko + (ci + 1) * CK)
        ka = src_ref[0:2 * T, cols].T
        kb = jnp.concatenate([src_ref[2 * T:3 * T, cols], src_ref[0:T, cols]], axis=0).T
        ka = pltpu.bitcast(ka, U32)
        kb = pltpu.bitcast(kb, U32)
        lane = lax.broadcasted_iota(I32, ka.shape, 1)
        rows = slice(ci * CK // 2, (ci + 1) * CK // 2)
        ka_ref[rows, :] = ka
        kb_ref[rows, :] = kb
        kc_ref[rows, :] = jnp.where(lane < T, kb, ka)

    def col_scales(src_ref, j):
        u = pltpu.bitcast(src_ref[:, j * BQ:(j + 1) * BQ], U32)
        hi = pltpu.bitcast(u & jnp.uint32(0xFFFF0000), F32)
        lo = pltpu.bitcast(lax.shift_left(u, jnp.uint32(16)), F32)
        ss = jnp.sum(hi * hi + lo * lo, axis=0, keepdims=True)
        ss = jnp.broadcast_to(ss, (8, BQ))
        e = lax.shift_right_logical(pltpu.bitcast(ss, I32), 24)
        up = pltpu.bitcast(lax.shift_left(190 - e, 23), F32)
        down = pltpu.bitcast(lax.shift_left(64 + e, 23), F32)
        return up, down * c

    def weight(src_ref, j, up, i):
        def part(half, t):
            cols = slice(j * BQ + half * hb, j * BQ + (half + 1) * hb)
            x = src_ref[t * T:(t + 1) * T, cols].astype(F32)
            u = up[:, half * hb:(half + 1) * hb]
            return (x.reshape(T // 8, 8, hb) * u[None]).reshape(T, hb)
        if i == 0:
            w = jnp.concatenate([part(1, 2), part(0, 1)], axis=0)
        elif i == 1:
            w = jnp.concatenate([part(0, 2) - part(1, 2), part(0, 0)], axis=0)
        else:
            w = jnp.concatenate([part(1, 0), part(1, 1) - part(0, 1)], axis=0)
        return w.astype(BF16)

    def a_chunk(ci, w, mrun):
        rows = slice(ci * CK // 2, (ci + 1) * CK // 2)
        p2 = jnp.dot(pltpu.bitcast(kb_ref[rows, :], BF16), w[1], preferred_element_type=F32)
        p1 = jnp.dot(pltpu.bitcast(kc_ref[rows, :], BF16), w[0], preferred_element_type=F32)
        p3 = jnp.dot(pltpu.bitcast(ka_ref[rows, :], BF16), w[2], preferred_element_type=F32)
        s = jnp.concatenate([p1 + p2, p1 + p3], axis=1)
        mm = jnp.max(s.reshape(CK // 8, 8, BQ), axis=0)
        return s, (mm if mrun is None else jnp.maximum(mrun, mm))

    def b_chunk(v_ref, ci, s, m8, c8, lrun, acc):
        p = jnp.exp2((s.reshape(CK // 8, 8, BQ) - m8[None]) * c8[None])
        ls = jnp.sum(p, axis=0)
        o = jnp.dot(v_ref[:, vo + ci * CK:vo + (ci + 1) * CK], p.reshape(CK, BQ).astype(BF16),
                    preferred_element_type=F32)
        return (ls if lrun is None else lrun + ls), (o if acc is None else acc + o)

    def col_max(mrun):
        return jnp.broadcast_to(jnp.max(mrun, axis=0, keepdims=True), (8, BQ))

    def order_after(m8, x):
        if x.dtype == I32:
            mi = pltpu.bitcast(m8, I32)
            return pltpu.bitcast(jnp.maximum(mi, jnp.minimum(x, mi)), F32)
        return jnp.maximum(m8, jnp.minimum(x, m8))

    def fold(w):
        u = jnp.max(pltpu.bitcast(w, I32).reshape(4, 16, hb), axis=0)
        return jnp.concatenate([u[:8], u[8:]], axis=1)

    def segment(ops, g0, g1, head_of, prep_next, out, resume):
        ms, ss, cs, scales, wnext = {}, {}, {}, {}, {}
        mhist, lhist, ahist, pend = [], [], [], []
        mrun = w = lrun = acc = None
        if resume:
            for i in range(LAG // nc):
                ms[g0 // nc + i] = mx_ref[i]
            for i in range(-(-LAG // nc)):
                cs[g0 // nc + i] = cx_ref[i]
            mrun = mx_ref[LAG // nc]
            w = tuple(pltpu.bitcast(wx_ref[i], BF16) for i in range(3))
        for op in ops:
            if op[0] == 'H':
                op[1]()
            elif op[0] == 'A':
                ga = op[1]
                blk, ci = divmod(ga, nc)
                if ci == 0:
                    if blk not in scales:
                        scales[blk] = col_scales(head_of(blk), blk % nq)
                    up, c8 = scales[blk]
                    w = tuple(wnext[i] if i in wnext else weight(head_of(blk), blk % nq, up, i)
                              for i in range(3))
                    wnext.clear()
                    if ga < g1:
                        cs[blk] = c8
                    else:
                        cx_ref[blk - g1 // nc] = c8
                    mrun = None
                if ci == PREP_AT and ('A', (blk + 1) * nc) in ops:
                    scales[blk + 1] = col_scales(head_of(blk + 1), (blk + 1) % nq)
                    pend.append(scales[blk + 1][1])
                i, r = divmod(ci - PREP_AT - PREP_GAP, PREP_GAP)
                if r == 0 and 0 <= i < 3 and (blk + 1) in scales:
                    wnext[i] = weight(head_of(blk + 1), (blk + 1) % nq, scales[blk + 1][0], i)
                    pend.append(fold(wnext[i]))
                s, mrun = a_chunk(ci, w, mrun)
                mhist.append(mrun)
                if ga < g1:
                    ss[ga] = s
                else:
                    sx_ref[ga - g1] = s
                if ci == nc - 1:
                    if ga < g1:
                        ms[blk] = col_max(mrun)
                    else:
                        mx_ref[blk - g1 // nc] = col_max(mrun)
                elif ga == g1 + LAG - 1:
                    mx_ref[blk - g1 // nc] = mrun
                    for i in range(3):
                        wx_ref[i] = pltpu.bitcast(w[i], U32)
                if blk == nq - 1 and prep_next:
                    k_prep(head_of(nq), ci)
            else:
                g, dacc, da = op[1:]
                blk, ci = divmod(g, nc)
                if ci == 0:
                    lrun = acc = None
                m8 = ms[blk]
                if da is not None and len(mhist) > da:
                    m8 = order_after(m8, mhist[-1 - da])
                if len(lhist) >= DL:
                    m8 = order_after(m8, lhist[-DL])
                while pend:
                    m8 = order_after(m8, pend.pop())
                if len(ahist) >= dacc:
                    m8 = order_after(m8, ahist[-dacc])
                s = ss.pop(g) if g in ss else sx_ref[g - g0]
                lrun, acc = b_chunk(head_of(blk), ci, s, m8, cs[blk], lrun, acc)
                lhist.append(lrun)
                ahist.append(acc[D - 8:D])
                if ci == nc - 1:
                    l = jnp.sum(lrun, axis=0, keepdims=True)
                    out(blk, (acc * (1.0 / l)).astype(BF16))

    q0 = ((LAG + LEAD - 1 - PREP_AT) // nc + 2) * BQ
    q1 = -(-(s0 + LAG) // nc) * BQ
    kp = Sk // 2

    def first_copy(src, off, lo, hi, i):
        return pltpu.make_async_copy(src.at[0, :, pl.ds(lo, hi - lo)],
                                     in_buf.at[0, :, pl.ds(off + lo, hi - lo)], sem_p.at[i])

    cp_q0 = first_copy(q_hbm, 0, 0, q0, 0)
    cp_q1 = first_copy(q_hbm, 0, q0, q1, 1)
    cp_q2 = first_copy(q_hbm, 0, q1, Sq, 6)
    cp_k = [first_copy(k_hbm, ko, i * kp, (i + 1) * kp, 3 + i) for i in range(2)]
    cp_v = first_copy(v_hbm, vo, 0, Sk, 5)
    cp_q0.start()
    cp_k[0].start()
    cp_k[1].start()
    cp_q0.wait()
    cp_v.start()
    cp_q1.start()

    def first_k(i):
        def f():
            if i == 1:
                cp_q2.start()
                for cp in head_copies(1, 1):
                    cp.start()
            cp_k[i].wait()
            for ci in range(i * nc // 2, (i + 1) * nc // 2):
                k_prep(in_buf.at[0], ci)
        return f

    def first_b():
        cp_q1.wait()
        cp_v.wait()

    def first_out(blk, val):
        o0_buf[:, blk * BQ:(blk + 1) * BQ] = val
        o_start(o0_buf.at[:, pl.ds(blk * BQ, BQ)], 0, blk, sem_p.at[2])

    ops = [('H', first_k(0))]
    for ga in range(LAG + LEAD):
        if ga == nc // 4:
            ops.append(('H', first_k(1)))
        ops.append(('A', ga))
    ops.append(('H', first_b))
    ga, g = LAG + LEAD, 0
    while g < s0:
        catch_up = ga - g > LAG
        ops.append(('A', ga))
        ops.append(('B', g, DACC_TAIL if catch_up else DACC, DA))
        ga, g = ga + 1, g + 1
        if catch_up:
            ops.append(('B', g, DACC_TAIL, DA))
            g += 1
    assert ga == s0 + LAG and g == s0
    segment(ops, 0, s0, lambda blk: in_buf.at[0], False, first_out, False)
    cp_q2.wait()
    wait_head(1)

    def step(h, carry):
        cur = h & 1
        oth = 1 - cur
        h1 = h + 1
        h2 = jnp.minimum(h + 2, BH - 1)
        i0, i1, i2 = h & 3, (h + 1) & 3, (h + 2) & 3

        def out(blk, val):
            pos = blk - SHIFT
            o_buf[cur, :, pos * BQ:(pos + 1) * BQ] = val
            o_start(o_buf.at[cur, :, pl.ds(pos * BQ, BQ)], h1 if blk >= nq else h, blk % nq,
                    sem_o.at[cur])

        fetch = dict(zip(FETCH_AT, head_copies(h2, i2)))
        ops = []
        for g in range(s0, total + s0):
            if g - s0 in fetch:
                ops.append(('H', fetch[g - s0].start))
            ops.append(('A', g + LAG))
            ops.append(('B', g, DACC, DA))
        segment(ops, s0, total + s0,
                lambda blk: in_buf.at[i1] if blk >= nq else in_buf.at[i0], True, out, True)

        @pl.when(h >= 1)
        def _():
            o_wait(oth, nq)

        wait_head(i2)
        return carry

    lax.fori_loop(0, nsteps, step, 0)

    cur = nsteps & 1

    def last_out(blk, val):
        pos = blk - SHIFT
        o_buf[cur, :, pos * BQ:(pos + 1) * BQ] = val
        o_start(o_buf.at[cur, :, pl.ds(pos * BQ, BQ)], BH - 1, blk, sem_o.at[cur])

    ops = []
    for g in range(s0, total):
        if g + LAG < total:
            ops.append(('A', g + LAG))
            ops.append(('B', g, DACC, DA))
        else:
            da = DA - (g + LAG - total + 1)
            ops.append(('B', g, DACC_TAIL, da if da >= 0 else None))
    segment(ops, s0, total, lambda blk: in_buf.at[nsteps & 3], False, last_out, True)
    pltpu.make_async_copy(o0_buf, o0_buf, sem_p.at[2]).wait()
    o_wait(1 - cur, nq)
    o_wait(cur, nq - SHIFT)


@jax.jit
def pallas_standalone__mha_softmax__prompt_kernel(
    q: jax.Array,
    k: jax.Array,
    v: jax.Array,
):
    B, H, Sq, D = q.shape
    Sk = k.shape[2]
    BH = B * H
    nc = Sk // CK
    nx = -(-LAG // nc)
    assert D == 192 and BH >= 3 and Sq % BQ == 0 and Sk % (2 * CK) == 0
    assert LAG % nc and nc > PREP_AT + 3 * PREP_GAP - 1 and SHIFT + nx < Sq // BQ
    qt = jnp.swapaxes(q, 2, 3).reshape(BH, D, Sq)
    kt = jnp.swapaxes(k, 2, 3).reshape(BH, D, Sk)
    vt = jnp.swapaxes(v, 2, 3).reshape(BH, D, Sk)
    ot = pl.pallas_call(
        functools.partial(_kernel, c=(D ** -0.5) * LOG2E),
        in_specs=[pl.BlockSpec(memory_space=pl.ANY)] * 3,
        out_specs=pl.BlockSpec(memory_space=pl.ANY),
        out_shape=jax.ShapeDtypeStruct((BH, D, Sq), q.dtype),
        scratch_shapes=[
            pltpu.VMEM((4, D, Sq + 2 * Sk), BF16),
            pltpu.VMEM((2, D, Sq), BF16),
            pltpu.VMEM((D, SHIFT * BQ), BF16),
            pltpu.VMEM((Sk // 2, 128), U32),
            pltpu.VMEM((Sk // 2, 128), U32),
            pltpu.VMEM((Sk // 2, 128), U32),
            pltpu.VMEM((LAG, CK, BQ), F32),
            pltpu.VMEM((nx, 8, BQ), F32),
            pltpu.VMEM((nx, 8, BQ), F32),
            pltpu.VMEM((3, 64, BQ // 2), U32),
            pltpu.SemaphoreType.DMA((4,)),
            pltpu.SemaphoreType.DMA((2,)),
            pltpu.SemaphoreType.DMA((7,)),
        ],
        compiler_params=pltpu.CompilerParams(vmem_limit_bytes=64 * 1024 * 1024),
    )(qt, kt, vt)
    return jnp.swapaxes(ot.reshape(B, H, D, Sq), 2, 3)
```

```python
import functools

import jax
import jax.numpy as jnp
from jax import lax
import jax.experimental.pallas as pl
import jax.experimental.pallas.tpu as pltpu

LOG2E = 1.4426950408889634
F32 = jnp.float32
BF16 = jnp.bfloat16
U32 = jnp.uint32
I32 = jnp.int32

BQ = 256
CK = 128
LAG = 18
SHIFT = 2
LEAD = 6
DA, DL, DACC, DACC_TAIL = 3, 2, 3, 5
PREP_AT, PREP_GAP = 9, 2
FETCH_AT = (2, 3, 4)


def _kernel(q_hbm, k_hbm, v_hbm, o_hbm,
            in_buf, o_buf, o0_buf, ka_ref, kb_ref, kc_ref,
            sx_ref, mx_ref, cx_ref, wx_ref,
            sem_in, sem_o, sem_p, *, c):
    BH, D, Sq = q_hbm.shape
    Sk = k_hbm.shape[2]
    T = D // 3
    hb = BQ // 2
    nq = Sq // BQ
    nc = Sk // CK
    total = nq * nc
    s0 = SHIFT * nc
    nsteps = BH - 1
    ko, vo = Sq, Sq + Sk

    def head_copies(head, slot):
        return [pltpu.make_async_copy(src.at[head], in_buf.at[slot, :, pl.ds(off, n)],
                                      sem_in.at[slot])
                for src, off, n in ((q_hbm, 0, Sq), (k_hbm, ko, Sk), (v_hbm, vo, Sk))]

    def wait_head(slot):
        pltpu.make_async_copy(in_buf.at[slot], in_buf.at[slot], sem_in.at[slot]).wait()

    def out_copy(h, slot, i):
        n0, n1 = Sq - SHIFT * BQ, SHIFT * BQ
        if i == 0:
            return pltpu.make_async_copy(o_buf.at[slot, :, pl.ds(0, n0)],
                                         o_hbm.at[h, :, pl.ds(n1, n0)], sem_o.at[2 * slot])
        return pltpu.make_async_copy(o_buf.at[slot, :, pl.ds(n0, n1)],
                                     o_hbm.at[h + 1, :, pl.ds(0, n1)], sem_o.at[2 * slot + 1])

    def k_prep(src_ref, ci):
        cols = slice(ko + ci * CK, ko + (ci + 1) * CK)
        ka = src_ref[0:2 * T, cols].T
        kb = jnp.concatenate([src_ref[2 * T:3 * T, cols], src_ref[0:T, cols]], axis=0).T
        ka = pltpu.bitcast(ka, U32)
        kb = pltpu.bitcast(kb, U32)
        lane = lax.broadcasted_iota(I32, ka.shape, 1)
        rows = slice(ci * CK // 2, (ci + 1) * CK // 2)
        ka_ref[rows, :] = ka
        kb_ref[rows, :] = kb
        kc_ref[rows, :] = jnp.where(lane < T, kb, ka)

    def col_scales(src_ref, j):
        u = pltpu.bitcast(src_ref[:, j * BQ:(j + 1) * BQ], U32)
        hi = pltpu.bitcast(u & jnp.uint32(0xFFFF0000), F32)
        lo = pltpu.bitcast(lax.shift_left(u, jnp.uint32(16)), F32)
        ss = jnp.sum(hi * hi + lo * lo, axis=0, keepdims=True)
        ss = jnp.broadcast_to(ss, (8, BQ))
        e = lax.shift_right_logical(pltpu.bitcast(ss, I32), 24)
        up = pltpu.bitcast(lax.shift_left(190 - e, 23), F32)
        down = pltpu.bitcast(lax.shift_left(64 + e, 23), F32)
        return up, down * c

    def weight(src_ref, j, up, i):
        def part(half, t):
            cols = slice(j * BQ + half * hb, j * BQ + (half + 1) * hb)
            x = src_ref[t * T:(t + 1) * T, cols].astype(F32)
            u = up[:, half * hb:(half + 1) * hb]
            return (x.reshape(T // 8, 8, hb) * u[None]).reshape(T, hb)
        if i == 0:
            w = jnp.concatenate([part(1, 2), part(0, 1)], axis=0)
        elif i == 1:
            w = jnp.concatenate([part(0, 2) - part(1, 2), part(0, 0)], axis=0)
        else:
            w = jnp.concatenate([part(1, 0), part(1, 1) - part(0, 1)], axis=0)
        return w.astype(BF16)

    def a_chunk(ci, w, mrun):
        rows = slice(ci * CK // 2, (ci + 1) * CK // 2)
        p2 = jnp.dot(pltpu.bitcast(kb_ref[rows, :], BF16), w[1], preferred_element_type=F32)
        p1 = jnp.dot(pltpu.bitcast(kc_ref[rows, :], BF16), w[0], preferred_element_type=F32)
        p3 = jnp.dot(pltpu.bitcast(ka_ref[rows, :], BF16), w[2], preferred_element_type=F32)
        s = jnp.concatenate([p1 + p2, p1 + p3], axis=1)
        mm = jnp.max(s.reshape(CK // 8, 8, BQ), axis=0)
        return s, (mm if mrun is None else jnp.maximum(mrun, mm))

    def b_chunk(v_ref, ci, s, m8, c8, lrun, acc):
        p = jnp.exp2((s.reshape(CK // 8, 8, BQ) - m8[None]) * c8[None])
        ls = jnp.sum(p, axis=0)
        o = jnp.dot(v_ref[:, vo + ci * CK:vo + (ci + 1) * CK], p.reshape(CK, BQ).astype(BF16),
                    preferred_element_type=F32)
        return (ls if lrun is None else lrun + ls), (o if acc is None else acc + o)

    def col_max(mrun):
        return jnp.broadcast_to(jnp.max(mrun, axis=0, keepdims=True), (8, BQ))

    def order_after(m8, x):
        if x.dtype == I32:
            mi = pltpu.bitcast(m8, I32)
            return pltpu.bitcast(jnp.maximum(mi, jnp.minimum(x, mi)), F32)
        return jnp.maximum(m8, jnp.minimum(x, m8))

    def fold(w):
        u = jnp.max(pltpu.bitcast(w, I32).reshape(4, 16, hb), axis=0)
        return jnp.concatenate([u[:8], u[8:]], axis=1)

    def segment(ops, g0, g1, head_of, prep_next, out, resume):
        ms, ss, cs, scales, wnext = {}, {}, {}, {}, {}
        mhist, lhist, ahist, pend = [], [], [], []
        mrun = w = lrun = acc = None
        if resume:
            for i in range(LAG // nc):
                ms[g0 // nc + i] = mx_ref[i]
            for i in range(-(-LAG // nc)):
                cs[g0 // nc + i] = cx_ref[i]
            mrun = mx_ref[LAG // nc]
            w = tuple(pltpu.bitcast(wx_ref[i], BF16) for i in range(3))
        for op in ops:
            if op[0] == 'H':
                op[1]()
            elif op[0] == 'A':
                ga = op[1]
                blk, ci = divmod(ga, nc)
                if ci == 0:
                    if blk not in scales:
                        scales[blk] = col_scales(head_of(blk), blk % nq)
                    up, c8 = scales[blk]
                    w = tuple(wnext[i] if i in wnext else weight(head_of(blk), blk % nq, up, i)
                              for i in range(3))
                    wnext.clear()
                    if ga < g1:
                        cs[blk] = c8
                    else:
                        cx_ref[blk - g1 // nc] = c8
                    mrun = None
                if ci == PREP_AT and ('A', (blk + 1) * nc) in ops:
                    scales[blk + 1] = col_scales(head_of(blk + 1), (blk + 1) % nq)
                    pend.append(scales[blk + 1][1])
                i, r = divmod(ci - PREP_AT - PREP_GAP, PREP_GAP)
                if r == 0 and 0 <= i < 3 and (blk + 1) in scales:
                    wnext[i] = weight(head_of(blk + 1), (blk + 1) % nq, scales[blk + 1][0], i)
                    pend.append(fold(wnext[i]))
                s, mrun = a_chunk(ci, w, mrun)
                mhist.append(mrun)
                if ga < g1:
                    ss[ga] = s
                else:
                    sx_ref[ga - g1] = s
                if ci == nc - 1:
                    if ga < g1:
                        ms[blk] = col_max(mrun)
                    else:
                        mx_ref[blk - g1 // nc] = col_max(mrun)
                elif ga == g1 + LAG - 1:
                    mx_ref[blk - g1 // nc] = mrun
                    for i in range(3):
                        wx_ref[i] = pltpu.bitcast(w[i], U32)
                if blk == nq - 1 and prep_next:
                    k_prep(head_of(nq), ci)
            else:
                g, dacc, da = op[1:]
                blk, ci = divmod(g, nc)
                if ci == 0:
                    lrun = acc = None
                m8 = ms[blk]
                if da is not None and len(mhist) > da:
                    m8 = order_after(m8, mhist[-1 - da])
                if len(lhist) >= DL:
                    m8 = order_after(m8, lhist[-DL])
                while pend:
                    m8 = order_after(m8, pend.pop())
                if len(ahist) >= dacc:
                    m8 = order_after(m8, ahist[-dacc])
                s = ss.pop(g) if g in ss else sx_ref[g - g0]
                lrun, acc = b_chunk(head_of(blk), ci, s, m8, cs[blk], lrun, acc)
                lhist.append(lrun)
                ahist.append(acc[D - 8:D])
                if ci == nc - 1:
                    l = jnp.sum(lrun, axis=0, keepdims=True)
                    out(blk, (acc * (1.0 / l)).astype(BF16))

    q0 = ((LAG + LEAD - 1 - PREP_AT) // nc + 2) * BQ
    q1 = -(-(s0 + LAG) // nc) * BQ
    kp = Sk // 2

    def first_copy(src, off, lo, hi, i):
        return pltpu.make_async_copy(src.at[0, :, pl.ds(lo, hi - lo)],
                                     in_buf.at[0, :, pl.ds(off + lo, hi - lo)], sem_p.at[i])

    cp_q0 = first_copy(q_hbm, 0, 0, q0, 0)
    cp_q1 = first_copy(q_hbm, 0, q0, q1, 1)
    cp_q2 = first_copy(q_hbm, 0, q1, Sq, 6)
    cp_k = [first_copy(k_hbm, ko, i * kp, (i + 1) * kp, 3 + i) for i in range(2)]
    cp_v = first_copy(v_hbm, vo, 0, Sk, 5)
    cp_q0.start()
    cp_k[0].start()
    cp_k[1].start()
    cp_q0.wait()
    cp_v.start()
    cp_q1.start()

    def first_k(i):
        def f():
            if i == 1:
                cp_q2.start()
                for cp in head_copies(1, 1):
                    cp.start()
            cp_k[i].wait()
            for ci in range(i * nc // 2, (i + 1) * nc // 2):
                k_prep(in_buf.at[0], ci)
        return f

    def first_b():
        cp_q1.wait()
        cp_v.wait()

    cp_o = pltpu.make_async_copy(o0_buf, o_hbm.at[0, :, pl.ds(0, SHIFT * BQ)], sem_p.at[2])

    def first_out(blk, val):
        o0_buf[:, blk * BQ:(blk + 1) * BQ] = val
        if blk == SHIFT - 1:
            cp_o.start()

    ops = [('H', first_k(0))]
    for ga in range(LAG + LEAD):
        if ga == nc // 4:
            ops.append(('H', first_k(1)))
        ops.append(('A', ga))
    ops.append(('H', first_b))
    ga, g = LAG + LEAD, 0
    while g < s0:
        catch_up = ga - g > LAG
        ops.append(('A', ga))
        ops.append(('B', g, DACC_TAIL if catch_up else DACC, DA))
        ga, g = ga + 1, g + 1
        if catch_up:
            ops.append(('B', g, DACC_TAIL, DA))
            g += 1
    assert ga == s0 + LAG and g == s0
    segment(ops, 0, s0, lambda blk: in_buf.at[0], False, first_out, False)
    cp_q2.wait()
    wait_head(1)

    def step(h, carry):
        cur = h & 1
        oth = 1 - cur
        h2 = jnp.minimum(h + 2, BH - 1)
        i0, i1, i2 = h & 3, (h + 1) & 3, (h + 2) & 3

        def out(blk, val):
            pos = blk - SHIFT
            o_buf[cur, :, pos * BQ:(pos + 1) * BQ] = val
            if blk == nq - 1:
                out_copy(h, cur, 0).start()
            if blk == nq + SHIFT - 1:
                out_copy(h, cur, 1).start()

        fetch = dict(zip(FETCH_AT, head_copies(h2, i2)))
        ops = []
        for g in range(s0, total + s0):
            if g - s0 in fetch:
                ops.append(('H', fetch[g - s0].start))
            ops.append(('A', g + LAG))
            ops.append(('B', g, DACC, DA))
        segment(ops, s0, total + s0,
                lambda blk: in_buf.at[i1] if blk >= nq else in_buf.at[i0], True, out, True)

        @pl.when(h >= 1)
        def _():
            out_copy(h - 1, oth, 0).wait()
            out_copy(h - 1, oth, 1).wait()

        wait_head(i2)
        return carry

    lax.fori_loop(0, nsteps, step, 0)

    cur = nsteps & 1

    nl = Sq - (SHIFT + 1) * BQ
    cp_l = {nq - 2: pltpu.make_async_copy(o_buf.at[cur, :, pl.ds(0, nl)],
                                          o_hbm.at[BH - 1, :, pl.ds(SHIFT * BQ, nl)],
                                          sem_o.at[2 * cur]),
            nq - 1: pltpu.make_async_copy(o_buf.at[cur, :, pl.ds(nl, BQ)],
                                          o_hbm.at[BH - 1, :, pl.ds(Sq - BQ, BQ)],
                                          sem_o.at[2 * cur + 1])}

    def last_out(blk, val):
        pos = blk - SHIFT
        o_buf[cur, :, pos * BQ:(pos + 1) * BQ] = val
        if blk in cp_l:
            cp_l[blk].start()

    ops = []
    for g in range(s0, total):
        if g + LAG < total:
            ops.append(('A', g + LAG))
            ops.append(('B', g, DACC, DA))
        else:
            da = DA - (g + LAG - total + 1)
            ops.append(('B', g, DACC_TAIL, da if da >= 0 else None))
    segment(ops, s0, total, lambda blk: in_buf.at[nsteps & 3], False, last_out, True)
    cp_o.wait()
    out_copy(nsteps - 1, 1 - cur, 0).wait()
    out_copy(nsteps - 1, 1 - cur, 1).wait()
    for cp in cp_l.values():
        cp.wait()


@jax.jit
def pallas_standalone__mha_softmax__prompt_kernel(
    q: jax.Array,
    k: jax.Array,
    v: jax.Array,
):
    B, H, Sq, D = q.shape
    Sk = k.shape[2]
    BH = B * H
    nc = Sk // CK
    nx = -(-LAG // nc)
    assert D == 192 and BH >= 3 and Sq % BQ == 0 and Sk % (2 * CK) == 0
    assert nc < LAG < 2 * nc and SHIFT + nx < Sq // BQ
    qt = jnp.swapaxes(q, 2, 3).reshape(BH, D, Sq)
    kt = jnp.swapaxes(k, 2, 3).reshape(BH, D, Sk)
    vt = jnp.swapaxes(v, 2, 3).reshape(BH, D, Sk)
    ot = pl.pallas_call(
        functools.partial(_kernel, c=(D ** -0.5) * LOG2E),
        in_specs=[pl.BlockSpec(memory_space=pl.ANY)] * 3,
        out_specs=pl.BlockSpec(memory_space=pl.ANY),
        out_shape=jax.ShapeDtypeStruct((BH, D, Sq), q.dtype),
        scratch_shapes=[
            pltpu.VMEM((4, D, Sq + 2 * Sk), BF16),
            pltpu.VMEM((2, D, Sq), BF16),
            pltpu.VMEM((D, SHIFT * BQ), BF16),
            pltpu.VMEM((Sk // 2, 128), U32),
            pltpu.VMEM((Sk // 2, 128), U32),
            pltpu.VMEM((Sk // 2, 128), U32),
            pltpu.VMEM((LAG, CK, BQ), F32),
            pltpu.VMEM((nx, 8, BQ), F32),
            pltpu.VMEM((nx, 8, BQ), F32),
            pltpu.VMEM((3, 64, BQ // 2), U32),
            pltpu.SemaphoreType.DMA((4,)),
            pltpu.SemaphoreType.DMA((4,)),
            pltpu.SemaphoreType.DMA((7,)),
        ],
        compiler_params=pltpu.CompilerParams(vmem_limit_bytes=64 * 1024 * 1024),
    )(qt, kt, vt)
    return jnp.swapaxes(ot.reshape(B, H, D, Sq), 2, 3)
```
